```python
import os as _os
_os.environ.setdefault("JAX_PLATFORMS", "cpu")
import jax
import jax.numpy as jnp

def _softmax(x, axis=-1):
    return jax.nn.softmax(x, axis=axis)
def _gelu(x):
    return jax.nn.gelu(x, approximate=True)
def _silu(x):
    return jax.nn.silu(x)
def _sigmoid(x):
    return jax.nn.sigmoid(x)
def _layernorm(x, axis=-1, eps=1e-5):
    m = jnp.mean(x, axis=axis, keepdims=True)
    v = jnp.var(x, axis=axis, keepdims=True)
    return (x - m) / jnp.sqrt(v + eps)
def _scatter_add(tgt, idx, src, axis=0):
    return tgt.at[idx].add(src)
def _segment_sum(src, seg, n):
    return jax.ops.segment_sum(src, seg, n)
class _Rng:
    def __init__(self, key):
        self._k = key
    def _next(self):
        self._k, sub = jax.random.split(self._k)
        return sub
    def normal(self, shape):
        return jax.random.normal(self._next(), shape, dtype=jnp.bfloat16)
    def randint(self, lo, hi, shape):
        return jax.random.randint(self._next(), shape, lo, hi, dtype=jnp.int32)
    def uniform(self, shape, lo=0.0, hi=1.0):
        return jax.random.uniform(self._next(), shape, jnp.bfloat16, lo, hi)
    def permutation(self, n):
        return jax.random.permutation(self._next(), n)


kernel_name = 'gated_mix__sliding_block_cached__swiglu_ffn__decode'

def setup_inputs():
    _rng = _Rng(jax.random.key(int.from_bytes(__import__("os").urandom(4), "little")))
    _w = (lambda a: (lambda t: t.astype(jnp.bfloat16) if jnp.issubdtype(t.dtype, jnp.floating) else t)(jnp.asarray(a)))
    def _A_setup():
        B, Sq, D = 1, 1, 512
        Hq, Hkv, Sk, Dh = 32, 32, 32768, 128
        assert Hq % Hkv == 0, (Hq, Hkv)
        return {
            "x": _w((lambda *s: _rng.normal(s) * 0.05)(B, Sq, D)),
            "k_cache": _w((lambda *s: _rng.normal(s) * 3.2)(B, Hkv, Sk, Dh)),
            "v_cache": _w((lambda *s: _rng.normal(s) * 1.6)(B, Hkv, Sk, Dh)),
            "wq": _w((lambda *s: _rng.normal(s) * 3.2)(D, Hq * Dh) * (D ** -0.5)),
            "wo": _w((lambda *s: _rng.normal(s) * 1.6)(Hq * Dh, D) * ((Hq * Dh) ** -0.5)),
        }
    _A_in = _A_setup()

    def _B_setup():
        B, S, D, F = 1, 1, 512, 1376
        return {
            "x": _w((lambda *s: _rng.normal(s) * 0.05)(B, S, D)),
            "w_gate": _w((lambda *s: _rng.normal(s) * 0.1)(D, F)),
            "w_up": _w((lambda *s: _rng.normal(s) * 0.1)(D, F)),
            "w_down": _w((lambda *s: _rng.normal(s) * 0.1)(F, D)),
        }
    _B_in = _B_setup()

    return {
        "A_x": _A_in["x"],
        "A_k_cache": _A_in["k_cache"],
        "A_v_cache": _A_in["v_cache"],
        "A_wq": _A_in["wq"],
        "A_wo": _A_in["wo"],
        "B_x": _B_in["x"],
        "B_w_gate": _B_in["w_gate"],
        "B_w_up": _B_in["w_up"],
        "B_w_down": _B_in["w_down"],
        "gate_w": _w((lambda *s: _rng.normal(s) * 0.05)(512) * 16.0),
    }

def reference(A_x, A_k_cache, A_v_cache, A_wq, A_wo, B_x, B_w_gate, B_w_up, B_w_down, gate_w):
    def _A_ref(x, k_cache, v_cache, wq, wo):
        B, Sq, D = x.shape
        Hq, Dh = 32, 128
        Hkv, Sk = k_cache.shape[1], k_cache.shape[2]
        W = min(4096, max(256, Sk // 4))
        rep = Hq // Hkv
        q = (lambda x, *d: x.transpose(*d))((x @ wq).reshape(B, Sq, Hq, Dh), 0, 2, 1, 3)
        k = jnp.repeat(k_cache[:, :, Sk - W:, :], rep, axis=1)
        v = jnp.repeat(v_cache[:, :, Sk - W:, :], rep, axis=1)
        scores = jnp.einsum("bhqd,bhkd->bhqk", q, k) * (Dh ** -0.5)
        p = _softmax(scores, axis=-1)
        o = jnp.einsum("bhqk,bhkd->bhqd", p, v)
        return (lambda x, *d: x.transpose(*d))(o, 0, 2, 1, 3).reshape(B, Sq, Hq * Dh) @ wo

    def _B_ref(x, w_gate, w_up, w_down):
        g = _silu(x @ w_gate)
        u = x @ w_up
        return (g * u) @ w_down

    x = A_x
    g = _sigmoid((x * gate_w).sum(-1, keepdims=True))
    a = _A_ref(x, A_k_cache, A_v_cache, A_wq, A_wo)
    b = _B_ref(x, B_w_gate, B_w_up, B_w_down)
    return g * a + (1 - g) * b
```

```python
import functools
import jax, jax.numpy as jnp
import jax.experimental.pallas as pl
import jax.experimental.pallas.tpu as pltpu

H=32; SK=32768; W=4096; DH=128; D=512; F=1376

def kernel(x_ref, k_ref, v_ref, wq_ref, wo_ref, wg_ref, wu_ref, wd_ref, gw_ref, o_ref, acc_ref):
    h = pl.program_id(0)
    x = x_ref[0]
    xb = jnp.broadcast_to(x, (8, D))
    @pl.when(h == 0)
    def _():
        g = jax.lax.dot_general(xb, wg_ref[...], (((1,), (1,)), ((), ())), preferred_element_type=jnp.float32)
        u = jax.lax.dot_general(xb, wu_ref[...], (((1,), (1,)), ((), ())), preferred_element_type=jnp.float32)
        hdn = (g * jax.nn.sigmoid(g)) * u
        b = jnp.dot(hdn.astype(jnp.bfloat16), wd_ref[...], preferred_element_type=jnp.float32)
        acc_ref[1] = b
        acc_ref[0] = jnp.zeros((8, D), jnp.float32)
    q = jnp.dot(xb, wq_ref[...], preferred_element_type=jnp.float32) * (DH ** -0.5)
    s = jax.lax.dot_general(q.astype(jnp.bfloat16), k_ref[0, 0], (((1,), (1,)), ((), ())), preferred_element_type=jnp.float32)
    m = jnp.max(s, axis=-1, keepdims=True)
    p = jnp.exp(s - m)
    l = jnp.sum(p, axis=-1, keepdims=True)
    o = jnp.dot(p.astype(jnp.bfloat16), v_ref[0, 0], preferred_element_type=jnp.float32) / l
    acc_ref[0] += jnp.dot(o.astype(jnp.bfloat16), wo_ref[...], preferred_element_type=jnp.float32)
    @pl.when(h == H - 1)
    def _():
        xf = x.astype(jnp.float32)
        gw = gw_ref[...].astype(jnp.float32)
        t = xf[:, 0:128] * gw[0:1] + xf[:, 128:256] * gw[1:2] + xf[:, 256:384] * gw[2:3] + xf[:, 384:512] * gw[3:4]
        gate = jax.nn.sigmoid(jnp.sum(t, axis=-1, keepdims=True))
        res = gate * acc_ref[0][0:1] + (1.0 - gate) * acc_ref[1][0:1]
        o_ref[0] = res.astype(o_ref.dtype)

@jax.jit
def pallas_gated_mix__sliding_block_cached__swiglu_ffn__decode_kernel(A_x, A_k_cache, A_v_cache, A_wq, A_wo, B_x, B_w_gate, B_w_up, B_w_down, gate_w):
    nb = SK // W
    return pl.pallas_call(kernel,
        grid=(H,),
        in_specs=[
            pl.BlockSpec((1,1,D), lambda h: (0,0,0)),
            pl.BlockSpec((1,1,W,DH), lambda h: (0,h,nb-1,0)),
            pl.BlockSpec((1,1,W,DH), lambda h: (0,h,nb-1,0)),
            pl.BlockSpec((D, DH), lambda h: (0,h)),
            pl.BlockSpec((DH, D), lambda h: (h,0)),
            pl.BlockSpec((F, D), lambda h: (0,0)),
            pl.BlockSpec((F, D), lambda h: (0,0)),
            pl.BlockSpec((F, D), lambda h: (0,0)),
            pl.BlockSpec((4, 128), lambda h: (0,0)),
        ],
        out_specs=pl.BlockSpec((1,1,D), lambda h: (0,0,0)),
        out_shape=jax.ShapeDtypeStruct((1,1,D), jnp.bfloat16),
        scratch_shapes=[pltpu.VMEM((2,8,D), jnp.float32)],
        compiler_params=pltpu.CompilerParams(dimension_semantics=("arbitrary",), vmem_limit_bytes=64*1024*1024),
    )(A_x, A_k_cache, A_v_cache, A_wq, A_wo, B_w_gate.T, B_w_up.T, B_w_down, gate_w.reshape(4,128))
```

```python
import functools, math
import jax, jax.numpy as jnp
from jax import lax
import jax.experimental.pallas as pl
import jax.experimental.pallas.tpu as pltpu

H=32; SK=32768; W=4096; DH=128; D=512; F=1376
LO, HI = 1, 0
SCALE_LOG2E = (DH ** -0.5) * math.log2(math.e)
NT = (((1,), (1,)), ((), ()))
HB = 4
QR = W // HB
FP = F // 4

def split(total, size):
    out = []; p = 0
    while p < total:
        s = min(size, total - p); out.append((p, s)); p += s
    return out

def make(R=40, at=(4, 13, 20), tail=(0, 1024, 1536, 1792, 1920, 2048), compute=True, flags=True, QKL=6, PVL=10, R0=40, NH0=0):
    ch = split(QR, R)
    NS = len(ch)
    fch = split(FP, R)
    ffn_items = [(a, r, n) for i in range(len(fch)) for a in range(3) for (r, n) in [fch[i]]]
    ntail = len(tail) - 1
    def kernel(x_hbm, k_hbm, v_hbm, wq_hbm, wo_hbm, wg_hbm, wu_hbm, wd_hbm, gw_hbm, o_ref,
               x_v, gw_v, kbuf, vbuf, wq_v, wo_v, wg_v, wu_v, wd_v, q_s, p_s, l_s, o_s, b_s, sems):
        S_WQ, S_K, S_V, S_F, S_WOH, S_WOL = 0, 1, 3, 5, 7, 8
        def wait_all(ref, sem):
            pltpu.make_async_copy(ref, ref, sem).wait()
        def kv_cp(src, dst, u, r, n, sem0):
            g = u // 4
            h0 = pl.multiple_of(g * HB, HB)
            r0 = pl.multiple_of((u % 4) * QR, QR) + r
            return pltpu.make_async_copy(src.at[0, pl.ds(h0, HB), pl.ds(SK - W + r0, n)], dst.at[pl.ds(h0, HB), pl.ds(r0, n)], sems.at[sem0 + g % 2])
        def row_cp(src, dst, r, n, sem):
            return pltpu.make_async_copy(src.at[pl.ds(r, n)], dst.at[pl.ds(r, n)], sem)

        def wq_start(i):
            r = pl.multiple_of((i // 8) * 8, 8); c = pl.multiple_of((i % 8) * 512, 512)
            pltpu.make_async_copy(wq_hbm.at[:, pl.ds(r, 8), pl.ds(c, 512)], wq_v.at[:, pl.ds(r, 8), pl.ds(c, 512)], sems.at[S_WQ]).start(priority=LO)
        def k0_start(rr, n):
            pltpu.make_async_copy(k_hbm.at[0, pl.ds(0, HB), pl.ds(SK - W + rr, n)], kbuf.at[pl.ds(0, HB), pl.ds(rr, n)], sems.at[S_K]).start(priority=HI)
        nk0 = -(-W // R0)
        PRE = 128 - nk0
        for i in range(PRE):
            wq_start(i)
            if i < NH0: k0_start(i * R0, R0)
        def l1(i, _):
            wq_start(PRE + i)
            k0_start(pl.multiple_of((i + NH0) * R0, 8), R0)
            return 0
        lax.fori_loop(0, W // R0 - NH0, l1, 0)
        for i in range(PRE + W // R0 - NH0, 128):
            wq_start(i)
        if W % R0: k0_start(W // R0 * R0, W % R0)
        xc = pltpu.make_async_copy(x_hbm, x_v, sems.at[S_WQ]); xc.start()
        gc = pltpu.make_async_copy(gw_hbm, gw_v, sems.at[S_WQ]); gc.start()

        def lo_tail_sem(r):
            for pi in range(ntail):
                if tail[pi] <= r < tail[pi + 1]: return S_WOL + pi
        def issue(j, s0, s1, last):
            @pl.when(j < 32)
            def _():
                for s in range(s0, s1):
                    r, n = ch[s]
                    kv_cp(v_hbm, vbuf, j - 4, r, n, S_V).start(priority=LO)
                    kv_cp(k_hbm, kbuf, j, r, n, S_K).start(priority=HI)
            @pl.when(j >= 32)
            def _():
                i = j - 32
                base = pl.multiple_of(i * FP, 8)
                for s in range(s0, len(ffn_items) if last else s1):
                    if s < NS:
                        r, n = ch[s]
                        kv_cp(v_hbm, vbuf, j - 4, r, n, S_V).start(priority=LO)
                    a, r, n = ffn_items[s]
                    src, dst = [(wg_hbm, wg_v), (wu_hbm, wu_v), (wd_hbm, wd_v)][a]
                    row_cp(src, dst, base + r, n, sems.at[S_F + i % 2]).start(priority=HI)

        def xb():
            return jnp.broadcast_to(x_v[0], (8, D))
        def qproj():
            xc.wait(); gc.wait(); wait_all(wq_v, sems.at[S_WQ])
            b_s[...] = jnp.zeros((8, D), jnp.float32)
            if not compute: return
            x8 = xb()
            q = jnp.dot(x8[:, 0:128], wq_v[0], preferred_element_type=jnp.float32)
            for t in range(1, 4):
                q = q + jnp.dot(x8[:, t * 128:(t + 1) * 128], wq_v[t], preferred_element_type=jnp.float32)
            q = q.astype(jnp.bfloat16)
            for hh in range(H):
                q_s[hh] = q[:, hh * DH:(hh + 1) * DH]
        def qk(h):
            @pl.when(h % 4 == 0)
            def _():
                wait_all(kbuf.at[pl.ds(pl.multiple_of(h, HB), HB)], sems.at[S_K + (h // 4) % 2])
            if not compute: return
            s = lax.dot_general(q_s[h], kbuf[h], NT, preferred_element_type=jnp.float32)
            m = jnp.max(s, axis=-1, keepdims=True)
            p = jnp.exp2((s - m) * SCALE_LOG2E)
            l_s[h] = jnp.broadcast_to(jnp.sum(p, axis=-1, keepdims=True), (8, DH))
            p_s[h] = p.astype(jnp.bfloat16)
        def pv_nowait(h):
            if not compute:
                o_s[h] = jnp.zeros((8, DH), jnp.bfloat16); return
            o = jnp.dot(p_s[h], vbuf[h], preferred_element_type=jnp.float32) / l_s[h]
            o_s[h] = o.astype(jnp.bfloat16)
        def pv(h):
            @pl.when(h % 4 == 0)
            def _():
                wait_all(vbuf.at[pl.ds(pl.multiple_of(h, HB), HB)], sems.at[S_V + (h // 4) % 2])
            pv_nowait(h)
        def ffn(i):
            base = pl.multiple_of(i * FP, 8)
            sl = pl.ds(base, FP)
            for ref in (wg_v, wu_v, wd_v):
                wait_all(ref.at[sl], sems.at[S_F + i % 2])
            if not compute: return
            x8 = xb()
            g = lax.dot_general(x8, wg_v[sl, :], NT, preferred_element_type=jnp.float32)
            u = lax.dot_general(x8, wu_v[sl, :], NT, preferred_element_type=jnp.float32)
            hd = (g * jax.nn.sigmoid(g) * u).astype(jnp.bfloat16)
            b_s[...] += jnp.dot(hd, wd_v[sl, :], preferred_element_type=jnp.float32)

        def body(j, _):
            issue(j, 0, at[0], False)
            pl.when(j >= QKL)(lambda: qk(j - QKL))
            issue(j, at[0], at[1], False)
            pl.when(j >= PVL)(lambda: pv(j - PVL))
            issue(j, at[1], at[2], False)
            pl.when(j == QKL - 1)(qproj)
            pl.when(j >= 33)(lambda: ffn(j - 33))
            issue(j, at[2], NS, True)
            return 0
        lax.fori_loop(4, 36, body, 0)

        lo_items = []
        for pi in range(ntail):
            lo_items += [(tail[pi] + r, n, S_WOL + pi) for r, n in split(tail[pi + 1] - tail[pi], R)]
        hi_items = [(2048 + r, n) for r, n in split(2048, R)]
        def issue_wo(s0, s1):
            for s in range(s0, s1):
                if s < len(lo_items):
                    r, n, si = lo_items[s]
                    row_cp(wo_hbm, wo_v, r, n, sems.at[si]).start(priority=LO)
                if s < len(hi_items):
                    r, n = hi_items[s]
                    row_cp(wo_hbm, wo_v, r, n, sems.at[S_WOH]).start(priority=HI)
        nfin = max(len(lo_items), len(hi_items))
        def fin(i, _):
            qk(36 - QKL + i)
            pv(36 - PVL + i)
            return 0
        issue_wo(0, 6)
        ffn(3)
        issue_wo(6, 12)
        seg = 12
        for h in range(36 - QKL, H):
            qk(h)
            issue_wo(seg, seg + 6); seg += 6
        for h in range(36 - PVL, 28):
            pv(h)
            issue_wo(seg, seg + 6); seg += 6
        issue_wo(seg, nfin)
        xf = x_v[0].astype(jnp.float32)
        gw = gw_v[...].astype(jnp.float32)
        t = xf[:, 0:128] * gw[0:1] + xf[:, 128:256] * gw[1:2] + xf[:, 256:384] * gw[2:3] + xf[:, 384:512] * gw[3:4]
        gate = jax.nn.sigmoid(jnp.sum(t, axis=-1, keepdims=True))
        wait_all(vbuf.at[pl.ds(28, HB)], sems.at[S_V + 1])
        for h in range(28, H):
            pv_nowait(h)
        def wo_proj(r0, r1):
            o = jnp.concatenate([o_s[h] for h in range(r0 // DH, r1 // DH)], axis=1)
            return jnp.dot(o, wo_v[r0:r1, :], preferred_element_type=jnp.float32)
        wait_all(wo_v.at[pl.ds(2048, 2048)], sems.at[S_WOH])
        res = (1.0 - gate) * b_s[...] + gate * wo_proj(2048, 4096)
        for pi in range(ntail):
            r0, r1 = tail[pi], tail[pi + 1]
            wait_all(wo_v.at[pl.ds(r0, r1 - r0)], sems.at[S_WOL + pi])
            res = res + gate * wo_proj(r0, r1)
        o_ref[0] = res[0:1].astype(o_ref.dtype)

    @jax.jit
    def f(A_x, A_k_cache, A_v_cache, A_wq, A_wo, B_x, B_w_gate, B_w_up, B_w_down, gate_w):
        bf = jnp.bfloat16
        return pl.pallas_call(kernel,
            in_specs=[pl.BlockSpec(memory_space=pl.ANY)] * 9,
            out_specs=pl.BlockSpec(memory_space=pltpu.VMEM),
            out_shape=jax.ShapeDtypeStruct((1,1,D), bf),
            scratch_shapes=[
                pltpu.VMEM((1,1,D), bf), pltpu.VMEM((4,128), bf),
                pltpu.VMEM((H, W, DH), bf), pltpu.VMEM((H, W, DH), bf),
                pltpu.VMEM((4, D // 4, H*DH), bf), pltpu.VMEM((H*DH, D), bf),
                pltpu.VMEM((F, D), bf), pltpu.VMEM((F, D), bf), pltpu.VMEM((F, D), bf),
                pltpu.VMEM((H, 8, DH), bf), pltpu.VMEM((H, 8, W), bf), pltpu.VMEM((H, 8, DH), jnp.float32),
                pltpu.VMEM((H, 8, DH), bf), pltpu.VMEM((8, D), jnp.float32),
                pltpu.SemaphoreType.DMA((8 + ntail,)),
            ],
            compiler_params=pltpu.CompilerParams(vmem_limit_bytes=100*1024*1024, disable_bounds_checks=flags, disable_semaphore_checks=flags),
        )(A_x, A_k_cache, A_v_cache, A_wq.reshape(4, D // 4, H*DH), A_wo, B_w_gate.T, B_w_up.T, B_w_down, gate_w.reshape(4,128))
    return f
pallas_gated_mix__sliding_block_cached__swiglu_ffn__decode_kernel = make()
```

```python
import functools
import math

import jax
import jax.numpy as jnp
from jax import lax
import jax.experimental.pallas as pl
import jax.experimental.pallas.tpu as pltpu

H = 32
DH = 128
D = 512
F = 1376
W = 4096
LO, HI = 1, 0
HB = 4
QR = W // HB
FP = F // 4
R = 40
QK_LAG = 6
PV_LAG = 10
AT = (4, 13, 20)
FIN_AT = (33, 40, 43, 46, 49)
TAIL = (0, 1024, 1536, 1792, 1920, 1984, 2024, 2048)
N_VPU = 3
SCALE_LOG2E = (DH ** -0.5) * math.log2(math.e)
NT = (((1,), (1,)), ((), ()))
S_WQ, S_K, S_V, S_F, S_WOH, S_WOL = 0, 1, 3, 5, 7, 9
N_SEM = S_WOL + len(TAIL) - 1


def _split(total, size):
    return [(p, min(size, total - p)) for p in range(0, total, size)]


def _kernel(x_hbm, k_hbm, v_hbm, wq_hbm, wo_hbm, wg_hbm, wu_hbm, wd_hbm, gw_hbm,
            o_ref,
            x_v, gw_v, kbuf, vbuf, wq_v, wo_v, wg_v, wu_v, wd_v,
            q_s, p_s, l_s, o_s, b_s, sems, *, row0):
    ch = _split(QR, R)
    n_slots = len(ch)
    ffn_items = [(a, r, n) for r, n in _split(FP, R) for a in range(3)]
    ffn_refs = ((wg_hbm, wg_v), (wu_hbm, wu_v), (wd_hbm, wd_v))
    n_tail = len(TAIL) - 1

    def wait_all(ref, sem):
        pltpu.make_async_copy(ref, ref, sems.at[sem]).wait()

    def kv_start(src, dst, u, r, n, sem0, prio):
        g = u // 4
        h0 = pl.multiple_of(g * HB, HB)
        r0 = pl.multiple_of((u % 4) * QR, QR) + r
        pltpu.make_async_copy(
            src.at[0, pl.ds(h0, HB), pl.ds(row0 + r0, n)],
            dst.at[pl.ds(h0, HB), pl.ds(r0, n)],
            sems.at[sem0 + g % 2]).start(priority=prio)

    def rows_start(src, dst, r, n, sem, prio):
        pltpu.make_async_copy(src.at[pl.ds(r, n)], dst.at[pl.ds(r, n)],
                              sems.at[sem]).start(priority=prio)

    def wq_start(i):
        r = pl.multiple_of((i // 8) * 8, 8)
        c = pl.multiple_of((i % 8) * 512, 512)
        pltpu.make_async_copy(wq_hbm.at[:, pl.ds(r, 8), pl.ds(c, 512)],
                              wq_v.at[:, pl.ds(r, 8), pl.ds(c, 512)],
                              sems.at[S_WQ]).start(priority=LO)

    def k0_start(r, n):
        pltpu.make_async_copy(k_hbm.at[0, pl.ds(0, HB), pl.ds(row0 + r, n)],
                              kbuf.at[pl.ds(0, HB), pl.ds(r, n)],
                              sems.at[S_K]).start(priority=HI)

    n_full = W // R
    pre = 128 - n_full - 1
    for i in range(pre):
        wq_start(i)

    def prologue(i, carry):
        wq_start(pre + i)
        k0_start(pl.multiple_of(i * R, 8), R)
        return carry

    lax.fori_loop(0, n_full, prologue, 0)
    wq_start(127)
    k0_start(n_full * R, W - n_full * R)
    x_cp = pltpu.make_async_copy(x_hbm, x_v, sems.at[S_WQ])
    gw_cp = pltpu.make_async_copy(gw_hbm, gw_v, sems.at[S_WQ])
    x_cp.start()
    gw_cp.start()

    def x8():
        return jnp.broadcast_to(x_v[0], (8, D))

    def q_proj():
        x_cp.wait()
        gw_cp.wait()
        wait_all(wq_v, S_WQ)
        b_s[...] = jnp.zeros((8, D), jnp.float32)
        x = x8()
        q = jnp.dot(x[:, 0:128], wq_v[0], preferred_element_type=jnp.float32)
        for t in range(1, 4):
            q = q + jnp.dot(x[:, t * 128:(t + 1) * 128], wq_v[t],
                            preferred_element_type=jnp.float32)
        q = q.astype(jnp.bfloat16)
        for h in range(H):
            q_s[h] = q[:, h * DH:(h + 1) * DH]

    def qk(h):
        @pl.when(h % HB == 0)
        def _():
            wait_all(kbuf.at[pl.ds(pl.multiple_of(h, HB), HB)],
                     S_K + (h // HB) % 2)

        s = lax.dot_general(q_s[h], kbuf[h], NT,
                            preferred_element_type=jnp.float32)
        m = jnp.max(s, axis=-1, keepdims=True)
        p = jnp.exp2((s - m) * SCALE_LOG2E)
        l_s[h] = jnp.broadcast_to(jnp.sum(p, axis=-1, keepdims=True), (8, DH))
        p_s[h] = p.astype(jnp.bfloat16)

    def pv(h):
        @pl.when(h % HB == 0)
        def _():
            wait_all(vbuf.at[pl.ds(pl.multiple_of(h, HB), HB)],
                     S_V + (h // HB) % 2)

        o = jnp.dot(p_s[h], vbuf[h], preferred_element_type=jnp.float32)
        o_s[h] = (o / l_s[h]).astype(jnp.bfloat16)

    def ffn(i):
        sl = pl.ds(pl.multiple_of(i * FP, 8), FP)
        for _, dst in ffn_refs:
            wait_all(dst.at[sl], S_F + i % 2)
        x = x8()
        g = lax.dot_general(x, wg_v[sl, :], NT,
                            preferred_element_type=jnp.float32)
        u = lax.dot_general(x, wu_v[sl, :], NT,
                            preferred_element_type=jnp.float32)
        hid = (g * jax.nn.sigmoid(g) * u).astype(jnp.bfloat16)
        b_s[...] += jnp.dot(hid, wd_v[sl, :],
                            preferred_element_type=jnp.float32)

    def issue(j, s0, s1):
        @pl.when(j < H)
        def _():
            for r, n in ch[s0:s1]:
                kv_start(v_hbm, vbuf, j - 4, r, n, S_V, LO)
                kv_start(k_hbm, kbuf, j, r, n, S_K, HI)

        @pl.when(j >= H)
        def _():
            i = j - H
            base = pl.multiple_of(i * FP, 8)
            for s in range(s0, len(ffn_items) if s1 == n_slots else s1):
                if s < n_slots:
                    kv_start(v_hbm, vbuf, j - 4, *ch[s], S_V, LO)
                a, r, n = ffn_items[s]
                rows_start(*ffn_refs[a], base + r, n, S_F + i % 2, HI)

    def body(j, carry):
        issue(j, 0, AT[0])
        pl.when(j >= QK_LAG)(lambda: qk(j - QK_LAG))
        issue(j, AT[0], AT[1])
        pl.when(j >= PV_LAG)(lambda: pv(j - PV_LAG))
        issue(j, AT[1], AT[2])
        pl.when(j == QK_LAG - 1)(q_proj)
        pl.when(j > H)(lambda: ffn(j - H - 1))
        issue(j, AT[2], n_slots)
        return carry

    lax.fori_loop(4, H + 4, body, 0)

    lo_items = [(TAIL[t] + r, n, S_WOL + t) for t in range(n_tail)
                for r, n in _split(TAIL[t + 1] - TAIL[t], R)]
    hi_items = [(2048 + 1024 * t + r, n, S_WOH + t) for t in range(2)
                for r, n in _split(1024, R)]
    n_fin = max(len(lo_items), len(hi_items))

    def issue_wo(s0, s1):
        for s in range(s0, s1):
            if s < len(lo_items):
                rows_start(wo_hbm, wo_v, *lo_items[s], LO)
            if s < len(hi_items):
                rows_start(wo_hbm, wo_v, *hi_items[s], HI)

    def wo_proj(r0, r1, sem):
        o = jnp.concatenate([o_s[h] for h in range(r0 // DH, r1 // DH)], axis=1)
        wait_all(wo_v.at[pl.ds(r0, r1 - r0)], sem)
        return jnp.dot(o, wo_v[r0:r1, :], preferred_element_type=jnp.float32)

    st = {}

    def mix_init():
        xf = x_v[0].astype(jnp.float32)
        gw = gw_v[...].astype(jnp.float32)
        t = xf[:, 0:128] * gw[0:1]
        for c in range(1, 4):
            t = t + xf[:, c * 128:(c + 1) * 128] * gw[c:c + 1]
        gate = jax.nn.sigmoid(jnp.sum(t, axis=-1, keepdims=True))
        st["gate"] = gate
        st["res"] = (1.0 - gate) * b_s[...] + gate * wo_proj(2048, 3072, S_WOH)

    acts = ([functools.partial(ffn, 3)]
            + [functools.partial(qk, h) for h in range(H + 4 - QK_LAG, H)]
            + [functools.partial(pv, h) for h in range(H + 4 - PV_LAG, H - HB)])
    acts = [(6 + 5 * i, a) for i, a in enumerate(acts)]
    acts += [(FIN_AT[0], mix_init)]
    acts += [(FIN_AT[1 + i], functools.partial(pv, H - HB + i))
             for i in range(HB)]
    done = 0
    for slot, act in acts:
        issue_wo(done, slot)
        done = slot
        act()
    issue_wo(done, n_fin)

    gate, res = st["gate"], st["res"]
    hv = TAIL[n_tail - N_VPU] // DH
    o_row = o_s[hv][0:1].astype(jnp.float32) * gate
    coef = jnp.transpose(jnp.broadcast_to(o_row, (DH, DH)))
    res = res + gate * wo_proj(3072, 4096, S_WOH + 1)
    for t in range(n_tail - N_VPU):
        res = res + gate * wo_proj(TAIL[t], TAIL[t + 1], S_WOL + t)
    acc = res * 0.125
    for t in range(n_tail - N_VPU, n_tail):
        wait_all(wo_v.at[pl.ds(TAIL[t], TAIL[t + 1] - TAIL[t])], S_WOL + t)
        for r in range(TAIL[t], TAIL[t + 1], 8):
            c = coef[r - hv * DH:r - hv * DH + 8]
            acc = acc + (wo_v[r:r + 8, :].astype(jnp.float32)
                         * jnp.concatenate([c, c, c, c], axis=1))
    o_ref[0] = jnp.sum(acc, axis=0, keepdims=True).astype(o_ref.dtype)


def _call(A_x, A_k_cache, A_v_cache, A_wq, A_wo, B_w_gate, B_w_up, B_w_down,
          gate_w, **kw):
    sk = A_k_cache.shape[2]
    assert A_x.shape == (1, 1, D) and A_k_cache.shape == (1, H, sk, DH)
    assert A_wq.shape == (D, H * DH) and B_w_gate.shape == (D, F)
    bf = jnp.bfloat16
    return pl.pallas_call(
        functools.partial(_kernel, row0=sk - W),
        in_specs=[pl.BlockSpec(memory_space=pl.ANY)] * 9,
        out_specs=pl.BlockSpec(memory_space=pltpu.VMEM),
        out_shape=jax.ShapeDtypeStruct((1, 1, D), A_x.dtype),
        scratch_shapes=[
            pltpu.VMEM((1, 1, D), bf),
            pltpu.VMEM((4, 128), bf),
            pltpu.VMEM((H, W, DH), bf),
            pltpu.VMEM((H, W, DH), bf),
            pltpu.VMEM((4, D // 4, H * DH), bf),
            pltpu.VMEM((H * DH, D), bf),
            pltpu.VMEM((F, D), bf),
            pltpu.VMEM((F, D), bf),
            pltpu.VMEM((F, D), bf),
            pltpu.VMEM((H, 8, DH), bf),
            pltpu.VMEM((H, 8, W), bf),
            pltpu.VMEM((H, 8, DH), jnp.float32),
            pltpu.VMEM((H, 8, DH), bf),
            pltpu.VMEM((8, D), jnp.float32),
            pltpu.SemaphoreType.DMA((N_SEM,)),
        ],
        compiler_params=pltpu.CompilerParams(
            vmem_limit_bytes=100 * 1024 * 1024,
            disable_bounds_checks=True,
            disable_semaphore_checks=True,
        ),
        **kw,
    )(A_x, A_k_cache, A_v_cache, A_wq.reshape(4, D // 4, H * DH), A_wo,
      B_w_gate.T, B_w_up.T, B_w_down, gate_w.reshape(4, 128))


@jax.jit
def pallas_gated_mix__sliding_block_cached__swiglu_ffn__decode_kernel(
    A_x: jax.Array,
    A_k_cache: jax.Array,
    A_v_cache: jax.Array,
    A_wq: jax.Array,
    A_wo: jax.Array,
    B_x: jax.Array,
    B_w_gate: jax.Array,
    B_w_up: jax.Array,
    B_w_down: jax.Array,
    gate_w: jax.Array,
):
    del B_x
    assert min(4096, max(256, A_k_cache.shape[2] // 4)) == W
    return _call(A_x, A_k_cache, A_v_cache, A_wq, A_wo, B_w_gate, B_w_up,
                 B_w_down, gate_w)
```

```python
import functools
import math

import jax
import jax.numpy as jnp
from jax import lax
import jax.experimental.pallas as pl
import jax.experimental.pallas.tpu as pltpu

H = 32
DH = 128
D = 512
F = 1376
W = 4096
LO, HI = 1, 0
HB = 4
QR = W // HB
FP = F // 4
R = 40
QK_LAG = 6
PV_LAG = 10
AT = (4, 13, 20)
FIN_AT = (33, 40, 43, 46, 49)
TAIL = (0, 1024, 1536, 1792, 1920, 2008, 2048)
N_VPU = 3
SCALE_LOG2E = (DH ** -0.5) * math.log2(math.e)
NT = (((1,), (1,)), ((), ()))
S_WQ, S_K, S_V, S_F, S_WOH, S_WOL = 0, 1, 3, 5, 7, 9
N_SEM = S_WOL + len(TAIL) - 1


def _split(total, size):
    return [(p, min(size, total - p)) for p in range(0, total, size)]


def _kernel(x_hbm, k_hbm, v_hbm, wq_hbm, wo_hbm, wg_hbm, wu_hbm, wd_hbm, gw_hbm,
            o_ref,
            x_v, gw_v, kbuf, vbuf, wq_v, wo_v, wg_v, wu_v, wd_v,
            q_s, p_s, l_s, o_s, b_s, sems, *, row0):
    ch = _split(QR, R)
    n_slots = len(ch)
    ffn_items = [(a, r, n) for r, n in _split(FP, R) for a in range(3)]
    ffn_refs = ((wg_hbm, wg_v), (wu_hbm, wu_v), (wd_hbm, wd_v))
    n_tail = len(TAIL) - 1

    def wait_all(ref, sem):
        pltpu.make_async_copy(ref, ref, sems.at[sem]).wait()

    def kv_start(src, dst, u, r, n, sem0, prio):
        g = u // 4
        h0 = pl.multiple_of(g * HB, HB)
        r0 = pl.multiple_of((u % 4) * QR, QR) + r
        pltpu.make_async_copy(
            src.at[0, pl.ds(h0, HB), pl.ds(row0 + r0, n)],
            dst.at[pl.ds(h0, HB), pl.ds(r0, n)],
            sems.at[sem0 + g % 2]).start(priority=prio)

    def rows_start(src, dst, r, n, sem, prio):
        pltpu.make_async_copy(src.at[pl.ds(r, n)], dst.at[pl.ds(r, n)],
                              sems.at[sem]).start(priority=prio)

    def wq_start(i):
        r = pl.multiple_of((i // 8) * 8, 8)
        c = pl.multiple_of((i % 8) * 512, 512)
        pltpu.make_async_copy(wq_hbm.at[:, pl.ds(r, 8), pl.ds(c, 512)],
                              wq_v.at[:, pl.ds(r, 8), pl.ds(c, 512)],
                              sems.at[S_WQ]).start(priority=LO)

    def k0_start(r, n):
        pltpu.make_async_copy(k_hbm.at[0, pl.ds(0, HB), pl.ds(row0 + r, n)],
                              kbuf.at[pl.ds(0, HB), pl.ds(r, n)],
                              sems.at[S_K]).start(priority=HI)

    n_full = W // R
    pre = 128 - n_full - 1
    for i in range(pre):
        wq_start(i)

    def prologue(i, carry):
        wq_start(pre + i)
        k0_start(pl.multiple_of(i * R, 8), R)
        return carry

    lax.fori_loop(0, n_full, prologue, 0)
    wq_start(127)
    k0_start(n_full * R, W - n_full * R)
    x_cp = pltpu.make_async_copy(x_hbm, x_v, sems.at[S_WQ])
    gw_cp = pltpu.make_async_copy(gw_hbm, gw_v, sems.at[S_WQ])
    x_cp.start()
    gw_cp.start()

    def x8():
        return jnp.broadcast_to(x_v[0], (8, D))

    def q_proj():
        x_cp.wait()
        gw_cp.wait()
        wait_all(wq_v, S_WQ)
        b_s[...] = jnp.zeros((8, D), jnp.float32)
        x = x8()
        q = jnp.dot(x[:, 0:128], wq_v[0], preferred_element_type=jnp.float32)
        for t in range(1, 4):
            q = q + jnp.dot(x[:, t * 128:(t + 1) * 128], wq_v[t],
                            preferred_element_type=jnp.float32)
        q = q.astype(jnp.bfloat16)
        for h in range(H):
            q_s[h] = q[:, h * DH:(h + 1) * DH]

    def qk(h):
        @pl.when(h % HB == 0)
        def _():
            wait_all(kbuf.at[pl.ds(pl.multiple_of(h, HB), HB)],
                     S_K + (h // HB) % 2)

        s = lax.dot_general(q_s[h], kbuf[h], NT,
                            preferred_element_type=jnp.float32)
        m = jnp.max(s, axis=-1, keepdims=True)
        p = jnp.exp2((s - m) * SCALE_LOG2E)
        l_s[h] = jnp.broadcast_to(jnp.sum(p, axis=-1, keepdims=True), (8, DH))
        p_s[h] = p.astype(jnp.bfloat16)

    def pv(h):
        @pl.when(h % HB == 0)
        def _():
            wait_all(vbuf.at[pl.ds(pl.multiple_of(h, HB), HB)],
                     S_V + (h // HB) % 2)

        o = jnp.dot(p_s[h], vbuf[h], preferred_element_type=jnp.float32)
        o_s[h] = (o / l_s[h]).astype(jnp.bfloat16)

    def ffn(i):
        sl = pl.ds(pl.multiple_of(i * FP, 8), FP)
        for _, dst in ffn_refs:
            wait_all(dst.at[sl], S_F + i % 2)
        x = x8()
        g = lax.dot_general(x, wg_v[sl, :], NT,
                            preferred_element_type=jnp.float32)
        u = lax.dot_general(x, wu_v[sl, :], NT,
                            preferred_element_type=jnp.float32)
        hid = (g * jax.nn.sigmoid(g) * u).astype(jnp.bfloat16)
        b_s[...] += jnp.dot(hid, wd_v[sl, :],
                            preferred_element_type=jnp.float32)

    def issue(j, s0, s1):
        @pl.when(j < H)
        def _():
            for r, n in ch[s0:s1]:
                kv_start(v_hbm, vbuf, j - 4, r, n, S_V, LO)
                kv_start(k_hbm, kbuf, j, r, n, S_K, HI)

        @pl.when(j >= H)
        def _():
            i = j - H
            base = pl.multiple_of(i * FP, 8)
            for s in range(s0, len(ffn_items) if s1 == n_slots else s1):
                if s < n_slots:
                    kv_start(v_hbm, vbuf, j - 4, *ch[s], S_V, LO)
                a, r, n = ffn_items[s]
                rows_start(*ffn_refs[a], base + r, n, S_F + i % 2, HI)

    def body(j, carry):
        issue(j, 0, AT[0])
        pl.when(j >= QK_LAG)(lambda: qk(j - QK_LAG))
        issue(j, AT[0], AT[1])
        pl.when(j >= PV_LAG)(lambda: pv(j - PV_LAG))
        issue(j, AT[1], AT[2])
        pl.when(j == QK_LAG - 1)(q_proj)
        pl.when(j > H)(lambda: ffn(j - H - 1))
        issue(j, AT[2], n_slots)
        return carry

    lax.fori_loop(4, H + 4, body, 0)

    lo_items = [(TAIL[t] + r, n, S_WOL + t) for t in range(n_tail)
                for r, n in _split(TAIL[t + 1] - TAIL[t], R)]
    hi_items = [(2048 + 1024 * t + r, n, S_WOH + t) for t in range(2)
                for r, n in _split(1024, R)]
    n_fin = max(len(lo_items), len(hi_items))

    def issue_wo(s0, s1):
        for s in range(s0, s1):
            if s < len(lo_items):
                rows_start(wo_hbm, wo_v, *lo_items[s], LO)
            if s < len(hi_items):
                rows_start(wo_hbm, wo_v, *hi_items[s], HI)

    def wo_proj(r0, r1, sem):
        o = jnp.concatenate([o_s[h] for h in range(r0 // DH, r1 // DH)], axis=1)
        wait_all(wo_v.at[pl.ds(r0, r1 - r0)], sem)
        return jnp.dot(o, wo_v[r0:r1, :], preferred_element_type=jnp.float32)

    st = {}

    def mix_init():
        xf = x_v[0].astype(jnp.float32)
        gw = gw_v[...].astype(jnp.float32)
        t = xf[:, 0:128] * gw[0:1]
        for c in range(1, 4):
            t = t + xf[:, c * 128:(c + 1) * 128] * gw[c:c + 1]
        gate = jax.nn.sigmoid(jnp.sum(t, axis=-1, keepdims=True))
        st["gate"] = gate
        st["res"] = (1.0 - gate) * b_s[...] + gate * wo_proj(2048, 3072, S_WOH)

    acts = ([functools.partial(ffn, 3)]
            + [functools.partial(qk, h) for h in range(H + 4 - QK_LAG, H)]
            + [functools.partial(pv, h) for h in range(H + 4 - PV_LAG, H - HB)])
    acts = [(6 + 5 * i, a) for i, a in enumerate(acts)]
    acts += [(FIN_AT[0], mix_init)]
    acts += [(FIN_AT[1 + i], functools.partial(pv, H - HB + i))
             for i in range(HB)]
    done = 0
    for slot, act in acts:
        issue_wo(done, slot)
        done = slot
        act()
    issue_wo(done, n_fin)

    gate, res = st["gate"], st["res"]
    rv = TAIL[n_tail - N_VPU]
    coef = jnp.concatenate([
        jnp.transpose(jnp.broadcast_to(
            o_s[h][0:1].astype(jnp.float32) * gate, (DH, DH)))
        for h in range(rv // DH, TAIL[n_tail] // DH)], axis=0)
    res = res + gate * wo_proj(3072, 4096, S_WOH + 1)
    for t in range(n_tail - N_VPU):
        res = res + gate * wo_proj(TAIL[t], TAIL[t + 1], S_WOL + t)
    acc = res * 0.125
    for t in range(n_tail - N_VPU, n_tail):
        wait_all(wo_v.at[pl.ds(TAIL[t], TAIL[t + 1] - TAIL[t])], S_WOL + t)
        for r in range(TAIL[t], TAIL[t + 1], 8):
            c = coef[r - rv:r - rv + 8]
            acc = acc + (wo_v[r:r + 8, :].astype(jnp.float32)
                         * jnp.concatenate([c, c, c, c], axis=1))
    o_ref[0] = jnp.sum(acc, axis=0, keepdims=True).astype(o_ref.dtype)


def _call(A_x, A_k_cache, A_v_cache, A_wq, A_wo, B_w_gate, B_w_up, B_w_down,
          gate_w, **kw):
    sk = A_k_cache.shape[2]
    assert A_x.shape == (1, 1, D) and A_k_cache.shape == (1, H, sk, DH)
    assert A_wq.shape == (D, H * DH) and B_w_gate.shape == (D, F)
    bf = jnp.bfloat16
    return pl.pallas_call(
        functools.partial(_kernel, row0=sk - W),
        in_specs=[pl.BlockSpec(memory_space=pl.ANY)] * 9,
        out_specs=pl.BlockSpec(memory_space=pltpu.VMEM),
        out_shape=jax.ShapeDtypeStruct((1, 1, D), A_x.dtype),
        scratch_shapes=[
            pltpu.VMEM((1, 1, D), bf),
            pltpu.VMEM((4, 128), bf),
            pltpu.VMEM((H, W, DH), bf),
            pltpu.VMEM((H, W, DH), bf),
            pltpu.VMEM((4, D // 4, H * DH), bf),
            pltpu.VMEM((H * DH, D), bf),
            pltpu.VMEM((F, D), bf),
            pltpu.VMEM((F, D), bf),
            pltpu.VMEM((F, D), bf),
            pltpu.VMEM((H, 8, DH), bf),
            pltpu.VMEM((H, 8, W), bf),
            pltpu.VMEM((H, 8, DH), jnp.float32),
            pltpu.VMEM((H, 8, DH), bf),
            pltpu.VMEM((8, D), jnp.float32),
            pltpu.SemaphoreType.DMA((N_SEM,)),
        ],
        compiler_params=pltpu.CompilerParams(
            vmem_limit_bytes=100 * 1024 * 1024,
            disable_bounds_checks=True,
            disable_semaphore_checks=True,
        ),
        **kw,
    )(A_x, A_k_cache, A_v_cache, A_wq.reshape(4, D // 4, H * DH), A_wo,
      B_w_gate.T, B_w_up.T, B_w_down, gate_w.reshape(4, 128))


@jax.jit
def pallas_gated_mix__sliding_block_cached__swiglu_ffn__decode_kernel(
    A_x: jax.Array,
    A_k_cache: jax.Array,
    A_v_cache: jax.Array,
    A_wq: jax.Array,
    A_wo: jax.Array,
    B_x: jax.Array,
    B_w_gate: jax.Array,
    B_w_up: jax.Array,
    B_w_down: jax.Array,
    gate_w: jax.Array,
):
    del B_x
    assert min(4096, max(256, A_k_cache.shape[2] // 4)) == W
    return _call(A_x, A_k_cache, A_v_cache, A_wq, A_wo, B_w_gate, B_w_up,
                 B_w_down, gate_w)
```

```python
import functools
import math

import jax
import jax.numpy as jnp
from jax import lax
import jax.experimental.pallas as pl
import jax.experimental.pallas.tpu as pltpu

H = 32
DH = 128
D = 512
F = 1376
W = 4096
LO, HI = 1, 0
HB = 4
QR = W // HB
FP = F // 4
R = 40
QK_LAG = 6
PV_LAG = 10
AT = (4, 13, 20)
TAIL = (0, 1024, 1536, 1792, 1920, 2008, 2048)
N_VPU = 3
SCALE_LOG2E = (DH ** -0.5) * math.log2(math.e)
NT = (((1,), (1,)), ((), ()))
S_WQ, S_K, S_V, S_F, S_WOH, S_WOL = 0, 1, 3, 5, 7, 9
N_SEM = S_WOL + len(TAIL) - 1


def _split(total, size):
    return [(p, min(size, total - p)) for p in range(0, total, size)]


def _kernel(x_hbm, k_hbm, v_hbm, wq_hbm, wo_hbm, wg_hbm, wu_hbm, wd_hbm, gw_hbm,
            o_ref,
            x_v, gw_v, kbuf, vbuf, wq_v, wo_v, wg_v, wu_v, wd_v,
            q_s, p_s, l_s, o_s, b_s, sems, *, row0):
    ch = _split(QR, R)
    n_slots = len(ch)
    ffn_items = [(a, r, n) for r, n in _split(FP, R) for a in range(3)]
    ffn_refs = ((wg_hbm, wg_v), (wu_hbm, wu_v), (wd_hbm, wd_v))
    n_tail = len(TAIL) - 1

    def wait_all(ref, sem):
        pltpu.make_async_copy(ref, ref, sems.at[sem]).wait()

    def kv_start(src, dst, u, r, n, sem0, prio):
        g = u // 4
        h0 = pl.multiple_of(g * HB, HB)
        r0 = pl.multiple_of((u % 4) * QR, QR) + r
        pltpu.make_async_copy(
            src.at[0, pl.ds(h0, HB), pl.ds(row0 + r0, n)],
            dst.at[pl.ds(h0, HB), pl.ds(r0, n)],
            sems.at[sem0 + g % 2]).start(priority=prio)

    def rows_start(src, dst, r, n, sem, prio):
        pltpu.make_async_copy(src.at[pl.ds(r, n)], dst.at[pl.ds(r, n)],
                              sems.at[sem]).start(priority=prio)

    def wq_start(i):
        r = pl.multiple_of((i // 8) * 8, 8)
        c = pl.multiple_of((i % 8) * 512, 512)
        pltpu.make_async_copy(wq_hbm.at[:, pl.ds(r, 8), pl.ds(c, 512)],
                              wq_v.at[:, pl.ds(r, 8), pl.ds(c, 512)],
                              sems.at[S_WQ]).start(priority=LO)

    def k0_start(r, n):
        pltpu.make_async_copy(k_hbm.at[0, pl.ds(0, HB), pl.ds(row0 + r, n)],
                              kbuf.at[pl.ds(0, HB), pl.ds(r, n)],
                              sems.at[S_K]).start(priority=HI)

    n_full = W // R
    pre = 128 - n_full - 1
    for i in range(pre):
        wq_start(i)

    def prologue(i, carry):
        wq_start(pre + i)
        k0_start(pl.multiple_of(i * R, 8), R)
        return carry

    lax.fori_loop(0, n_full, prologue, 0)
    wq_start(127)
    k0_start(n_full * R, W - n_full * R)
    x_cp = pltpu.make_async_copy(x_hbm, x_v, sems.at[S_WQ])
    gw_cp = pltpu.make_async_copy(gw_hbm, gw_v, sems.at[S_WQ])
    x_cp.start()
    gw_cp.start()

    def x8():
        return jnp.broadcast_to(x_v[0], (8, D))

    def q_proj():
        x_cp.wait()
        gw_cp.wait()
        wait_all(wq_v, S_WQ)
        b_s[...] = jnp.zeros((8, D), jnp.float32)
        x = x8()
        q = jnp.dot(x[:, 0:128], wq_v[0], preferred_element_type=jnp.float32)
        for t in range(1, 4):
            q = q + jnp.dot(x[:, t * 128:(t + 1) * 128], wq_v[t],
                            preferred_element_type=jnp.float32)
        q = q.astype(jnp.bfloat16)
        for h in range(H):
            q_s[h] = q[:, h * DH:(h + 1) * DH]

    def qk(h):
        @pl.when(h % HB == 0)
        def _():
            wait_all(kbuf.at[pl.ds(pl.multiple_of(h, HB), HB)],
                     S_K + (h // HB) % 2)

        s = lax.dot_general(q_s[h], kbuf[h], NT,
                            preferred_element_type=jnp.float32)
        m = jnp.max(s, axis=-1, keepdims=True)
        p = jnp.exp2((s - m) * SCALE_LOG2E)
        l_s[h] = jnp.broadcast_to(jnp.sum(p, axis=-1, keepdims=True), (8, DH))
        p_s[h] = p.astype(jnp.bfloat16)

    def pv(h):
        @pl.when(h % HB == 0)
        def _():
            wait_all(vbuf.at[pl.ds(pl.multiple_of(h, HB), HB)],
                     S_V + (h // HB) % 2)

        o = jnp.dot(p_s[h], vbuf[h], preferred_element_type=jnp.float32)
        o_s[h] = (o / l_s[h]).astype(jnp.bfloat16)

    def ffn(i):
        sl = pl.ds(pl.multiple_of(i * FP, 8), FP)
        for _, dst in ffn_refs:
            wait_all(dst.at[sl], S_F + i % 2)
        x = x8()
        g = lax.dot_general(x, wg_v[sl, :], NT,
                            preferred_element_type=jnp.float32)
        u = lax.dot_general(x, wu_v[sl, :], NT,
                            preferred_element_type=jnp.float32)
        hid = (g * jax.nn.sigmoid(g) * u).astype(jnp.bfloat16)
        b_s[...] += jnp.dot(hid, wd_v[sl, :],
                            preferred_element_type=jnp.float32)

    def issue(j, s0, s1):
        @pl.when(j < H)
        def _():
            for r, n in ch[s0:s1]:
                kv_start(v_hbm, vbuf, j - 4, r, n, S_V, LO)
                kv_start(k_hbm, kbuf, j, r, n, S_K, HI)

        @pl.when(j >= H)
        def _():
            i = j - H
            base = pl.multiple_of(i * FP, 8)
            for s in range(s0, len(ffn_items) if s1 == n_slots else s1):
                if s < n_slots:
                    kv_start(v_hbm, vbuf, j - 4, *ch[s], S_V, LO)
                a, r, n = ffn_items[s]
                rows_start(*ffn_refs[a], base + r, n, S_F + i % 2, HI)

    def body(j, carry):
        issue(j, 0, AT[0])
        pl.when(j >= QK_LAG)(lambda: qk(j - QK_LAG))
        issue(j, AT[0], AT[1])
        pl.when(j >= PV_LAG)(lambda: pv(j - PV_LAG))
        issue(j, AT[1], AT[2])
        pl.when(j == QK_LAG - 1)(q_proj)
        pl.when(j > H)(lambda: ffn(j - H - 1))
        issue(j, AT[2], n_slots)
        return carry

    lax.fori_loop(4, H + 4, body, 0)

    lo_items = [(TAIL[t] + r, n, S_WOL + t) for t in range(n_tail)
                for r, n in _split(TAIL[t + 1] - TAIL[t], R)]
    hi_items = [(2048 + 1024 * t + r, n, S_WOH + t) for t in range(2)
                for r, n in _split(1024, R)]
    n_fin = max(len(lo_items), len(hi_items))

    def issue_wo(s0, s1):
        for s in range(s0, s1):
            if s < len(lo_items):
                rows_start(wo_hbm, wo_v, *lo_items[s], LO)
            if s < len(hi_items):
                rows_start(wo_hbm, wo_v, *hi_items[s], HI)

    def wo_proj(r0, r1, sem):
        o = jnp.concatenate([o_s[h] for h in range(r0 // DH, r1 // DH)], axis=1)
        wait_all(wo_v.at[pl.ds(r0, r1 - r0)], sem)
        return jnp.dot(o, wo_v[r0:r1, :], preferred_element_type=jnp.float32)

    st = {}

    def mix_init():
        xf = x_v[0].astype(jnp.float32)
        gw = gw_v[...].astype(jnp.float32)
        t = xf[:, 0:128] * gw[0:1]
        for c in range(1, 4):
            t = t + xf[:, c * 128:(c + 1) * 128] * gw[c:c + 1]
        gate = jax.nn.sigmoid(jnp.sum(t, axis=-1, keepdims=True))
        st["gate"] = gate
        st["res"] = (1.0 - gate) * b_s[...] + gate * wo_proj(2048, 3072, S_WOH)

    acts = ([functools.partial(ffn, 3)]
            + [functools.partial(qk, h) for h in range(H + 4 - QK_LAG, H)]
            + [functools.partial(pv, h) for h in range(H + 4 - PV_LAG, H - HB)])
    acts = [(6 + 5 * i, a) for i, a in enumerate(acts)]
    acts += [(33, mix_init)]
    done = 0
    for slot, act in acts:
        assert done <= slot <= n_fin
        issue_wo(done, slot)
        done = slot
        act()
    issue_wo(done, n_fin)
    for h in range(H - HB, H):
        pv(h)

    gate, res = st["gate"], st["res"]
    rv = TAIL[n_tail - N_VPU]
    coef = jnp.concatenate([
        jnp.transpose(jnp.broadcast_to(
            o_s[h][0:1].astype(jnp.float32) * gate, (DH, DH)))
        for h in range(rv // DH, TAIL[n_tail] // DH)], axis=0)
    res = res + gate * wo_proj(3072, 4096, S_WOH + 1)
    for t in range(n_tail - N_VPU):
        res = res + gate * wo_proj(TAIL[t], TAIL[t + 1], S_WOL + t)
    acc = res * 0.125
    for t in range(n_tail - N_VPU, n_tail):
        wait_all(wo_v.at[pl.ds(TAIL[t], TAIL[t + 1] - TAIL[t])], S_WOL + t)
        for r in range(TAIL[t], TAIL[t + 1], 8):
            c = coef[r - rv:r - rv + 8]
            acc = acc + (wo_v[r:r + 8, :].astype(jnp.float32)
                         * jnp.concatenate([c, c, c, c], axis=1))
    o_ref[0] = jnp.sum(acc, axis=0, keepdims=True).astype(o_ref.dtype)


def _call(A_x, A_k_cache, A_v_cache, A_wq, A_wo, B_w_gate, B_w_up, B_w_down,
          gate_w, **kw):
    sk = A_k_cache.shape[2]
    assert A_x.shape == (1, 1, D) and A_k_cache.shape == (1, H, sk, DH)
    assert A_wq.shape == (D, H * DH) and B_w_gate.shape == (D, F)
    bf = jnp.bfloat16
    return pl.pallas_call(
        functools.partial(_kernel, row0=sk - W),
        in_specs=[pl.BlockSpec(memory_space=pl.ANY)] * 9,
        out_specs=pl.BlockSpec(memory_space=pltpu.VMEM),
        out_shape=jax.ShapeDtypeStruct((1, 1, D), A_x.dtype),
        scratch_shapes=[
            pltpu.VMEM((1, 1, D), bf),
            pltpu.VMEM((4, 128), bf),
            pltpu.VMEM((H, W, DH), bf),
            pltpu.VMEM((H, W, DH), bf),
            pltpu.VMEM((4, D // 4, H * DH), bf),
            pltpu.VMEM((H * DH, D), bf),
            pltpu.VMEM((F, D), bf),
            pltpu.VMEM((F, D), bf),
            pltpu.VMEM((F, D), bf),
            pltpu.VMEM((H, 8, DH), bf),
            pltpu.VMEM((H, 8, W), bf),
            pltpu.VMEM((H, 8, DH), jnp.float32),
            pltpu.VMEM((H, 8, DH), bf),
            pltpu.VMEM((8, D), jnp.float32),
            pltpu.SemaphoreType.DMA((N_SEM,)),
        ],
        compiler_params=pltpu.CompilerParams(
            vmem_limit_bytes=100 * 1024 * 1024,
            disable_semaphore_checks=True,
        ),
        **kw,
    )(A_x, A_k_cache, A_v_cache, A_wq.reshape(4, D // 4, H * DH), A_wo,
      B_w_gate.T, B_w_up.T, B_w_down, gate_w.reshape(4, 128))


@jax.jit
def pallas_gated_mix__sliding_block_cached__swiglu_ffn__decode_kernel(
    A_x: jax.Array,
    A_k_cache: jax.Array,
    A_v_cache: jax.Array,
    A_wq: jax.Array,
    A_wo: jax.Array,
    B_x: jax.Array,
    B_w_gate: jax.Array,
    B_w_up: jax.Array,
    B_w_down: jax.Array,
    gate_w: jax.Array,
):
    del B_x
    assert min(4096, max(256, A_k_cache.shape[2] // 4)) == W
    return _call(A_x, A_k_cache, A_v_cache, A_wq, A_wo, B_w_gate, B_w_up,
                 B_w_down, gate_w)
```

```python
import functools
import math

import jax
import jax.numpy as jnp
from jax import lax
import jax.experimental.pallas as pl
import jax.experimental.pallas.tpu as pltpu

H = 32
DH = 128
D = 512
F = 1376
W = 4096
LO, HI = 1, 0
HB = 4
QR = W // HB
FP = F // 4
R = 40
KV_ROWS = ([40] * 7 + [48]) * 3 + [40]
V_ROT = 3
QK_LAG = 6
PV_LAG = 10
AT = (4, 13, 20)
TAIL = (0, 1024, 1536, 1792, 1920, 2008, 2048)
N_VPU = 3
SCALE_LOG2E = (DH ** -0.5) * math.log2(math.e)
NT = (((1,), (1,)), ((), ()))
S_WQ, S_K, S_V, S_F, S_WOH, S_WOL = 0, 1, 3, 5, 7, 9
N_SEM = S_WOL + len(TAIL) - 1


def _split(total, size):
    return [(p, min(size, total - p)) for p in range(0, total, size)]


def _kernel(x_hbm, k_hbm, v_hbm, wq_hbm, wo_hbm, wg_hbm, wu_hbm, wd_hbm, gw_hbm,
            o_ref,
            x_v, gw_v, kbuf, vbuf, wq_v, wo_v, wg_v, wu_v, wd_v,
            q_s, p_s, l_s, o_s, b_s, sems, *, row0):
    assert sum(KV_ROWS) == QR
    ch = [(sum(KV_ROWS[:i]), n) for i, n in enumerate(KV_ROWS)]
    n_slots = len(ch)
    ffn_items = [(a, r, n) for r, n in _split(FP, R) for a in range(3)]
    assert len(ffn_items) >= n_slots
    ffn_refs = ((wg_hbm, wg_v), (wu_hbm, wu_v), (wd_hbm, wd_v))
    n_tail = len(TAIL) - 1

    def wait_all(ref, sem):
        pltpu.make_async_copy(ref, ref, sems.at[sem]).wait()

    def kv_start(src, dst, u, rot, r, n, sem0, prio):
        g = u // 4
        h0 = pl.multiple_of(g * HB, HB)
        r0 = pl.multiple_of(((u + rot) % 4) * QR, QR) + r
        pltpu.make_async_copy(
            src.at[0, pl.ds(h0, HB), pl.ds(row0 + r0, n)],
            dst.at[pl.ds(h0, HB), pl.ds(r0, n)],
            sems.at[sem0 + g % 2]).start(priority=prio)

    def rows_start(src, dst, r, n, sem, prio):
        pltpu.make_async_copy(src.at[pl.ds(r, n)], dst.at[pl.ds(r, n)],
                              sems.at[sem]).start(priority=prio)

    def wq_start(i):
        r = pl.multiple_of((i // 8) * 8, 8)
        c = pl.multiple_of((i % 8) * 512, 512)
        pltpu.make_async_copy(wq_hbm.at[:, pl.ds(r, 8), pl.ds(c, 512)],
                              wq_v.at[:, pl.ds(r, 8), pl.ds(c, 512)],
                              sems.at[S_WQ]).start(priority=LO)

    def k0_start(r, n):
        pltpu.make_async_copy(k_hbm.at[0, pl.ds(0, HB), pl.ds(row0 + r, n)],
                              kbuf.at[pl.ds(0, HB), pl.ds(r, n)],
                              sems.at[S_K]).start(priority=HI)

    n_full = W // R
    pre = 128 - n_full - 1
    for i in range(pre):
        wq_start(i)

    def prologue(i, carry):
        wq_start(pre + i)
        k0_start(pl.multiple_of(i * R, 8), R)
        return carry

    lax.fori_loop(0, n_full, prologue, 0)
    wq_start(127)
    k0_start(n_full * R, W - n_full * R)
    x_cp = pltpu.make_async_copy(x_hbm, x_v, sems.at[S_WQ])
    gw_cp = pltpu.make_async_copy(gw_hbm, gw_v, sems.at[S_WQ])
    x_cp.start()
    gw_cp.start()

    def x8():
        return jnp.broadcast_to(x_v[0], (8, D))

    def q_proj():
        x_cp.wait()
        gw_cp.wait()
        wait_all(wq_v, S_WQ)
        b_s[...] = jnp.zeros((8, D), jnp.float32)
        x = x8()
        q = jnp.dot(x[:, 0:128], wq_v[0], preferred_element_type=jnp.float32)
        for t in range(1, 4):
            q = q + jnp.dot(x[:, t * 128:(t + 1) * 128], wq_v[t],
                            preferred_element_type=jnp.float32)
        q = q.astype(jnp.bfloat16)
        for h in range(H):
            q_s[h] = q[:, h * DH:(h + 1) * DH]

    def qk(h):
        @pl.when(h % HB == 0)
        def _():
            wait_all(kbuf.at[pl.ds(pl.multiple_of(h, HB), HB)],
                     S_K + (h // HB) % 2)

        s = lax.dot_general(q_s[h], kbuf[h], NT,
                            preferred_element_type=jnp.float32)
        m = jnp.max(s, axis=-1, keepdims=True)
        p = jnp.exp2((s - m) * SCALE_LOG2E)
        l_s[h] = jnp.broadcast_to(jnp.sum(p, axis=-1, keepdims=True), (8, DH))
        p_s[h] = p.astype(jnp.bfloat16)

    def pv(h):
        @pl.when(h % HB == 0)
        def _():
            wait_all(vbuf.at[pl.ds(pl.multiple_of(h, HB), HB)],
                     S_V + (h // HB) % 2)

        o = jnp.dot(p_s[h], vbuf[h], preferred_element_type=jnp.float32)
        o_s[h] = (o / l_s[h]).astype(jnp.bfloat16)

    def ffn(i):
        sl = pl.ds(pl.multiple_of(i * FP, 8), FP)
        for _, dst in ffn_refs:
            wait_all(dst.at[sl], S_F + i % 2)
        x = x8()
        g = lax.dot_general(x, wg_v[sl, :], NT,
                            preferred_element_type=jnp.float32)
        u = lax.dot_general(x, wu_v[sl, :], NT,
                            preferred_element_type=jnp.float32)
        hid = (g * jax.nn.sigmoid(g) * u).astype(jnp.bfloat16)
        b_s[...] += jnp.dot(hid, wd_v[sl, :],
                            preferred_element_type=jnp.float32)

    def issue(j, s0, s1):
        @pl.when(j < H)
        def _():
            for r, n in ch[s0:s1]:
                kv_start(v_hbm, vbuf, j - 4, V_ROT, r, n, S_V, LO)
                kv_start(k_hbm, kbuf, j, 0, r, n, S_K, HI)

        @pl.when(j >= H)
        def _():
            i = j - H
            base = pl.multiple_of(i * FP, 8)
            for s in range(s0, len(ffn_items) if s1 == n_slots else s1):
                if s < n_slots:
                    kv_start(v_hbm, vbuf, j - 4, V_ROT, *ch[s], S_V, LO)
                a, r, n = ffn_items[s]
                rows_start(*ffn_refs[a], base + r, n, S_F + i % 2, HI)

    def body(j, carry):
        issue(j, 0, AT[0])
        pl.when(j >= QK_LAG)(lambda: qk(j - QK_LAG))
        issue(j, AT[0], AT[1])
        pl.when(j >= PV_LAG)(lambda: pv(j - PV_LAG))
        issue(j, AT[1], AT[2])
        pl.when(j == QK_LAG - 1)(q_proj)
        pl.when(j > H)(lambda: ffn(j - H - 1))
        issue(j, AT[2], n_slots)
        return carry

    lax.fori_loop(4, H + 4, body, 0)

    lo_items = [(TAIL[t] + r, n, S_WOL + t) for t in range(n_tail)
                for r, n in _split(TAIL[t + 1] - TAIL[t], R)]
    hi_items = [(2048 + 1024 * t + r, n, S_WOH + t) for t in range(2)
                for r, n in _split(1024, R)]
    n_fin = max(len(lo_items), len(hi_items))

    def issue_wo(s0, s1):
        for s in range(s0, s1):
            if s < len(lo_items):
                rows_start(wo_hbm, wo_v, *lo_items[s], LO)
            if s < len(hi_items):
                rows_start(wo_hbm, wo_v, *hi_items[s], HI)

    def wo_proj(r0, r1, sem):
        o = jnp.concatenate([o_s[h] for h in range(r0 // DH, r1 // DH)], axis=1)
        wait_all(wo_v.at[pl.ds(r0, r1 - r0)], sem)
        return jnp.dot(o, wo_v[r0:r1, :], preferred_element_type=jnp.float32)

    st = {}

    def mix_init():
        xf = x_v[0].astype(jnp.float32)
        gw = gw_v[...].astype(jnp.float32)
        t = xf[:, 0:128] * gw[0:1]
        for c in range(1, 4):
            t = t + xf[:, c * 128:(c + 1) * 128] * gw[c:c + 1]
        gate = jax.nn.sigmoid(jnp.sum(t, axis=-1, keepdims=True))
        st["gate"] = gate
        st["res"] = (1.0 - gate) * b_s[...] + gate * wo_proj(2048, 3072, S_WOH)

    acts = ([functools.partial(ffn, 3)]
            + [functools.partial(qk, h) for h in range(H + 4 - QK_LAG, H)]
            + [functools.partial(pv, h) for h in range(H + 4 - PV_LAG, H - HB)])
    acts = [(6 + 5 * i, a) for i, a in enumerate(acts)]
    acts += [(33, mix_init)]
    done = 0
    for slot, act in acts:
        assert done <= slot <= n_fin
        issue_wo(done, slot)
        done = slot
        act()
    issue_wo(done, n_fin)
    for h in range(H - HB, H):
        pv(h)

    gate, res = st["gate"], st["res"]
    rv = TAIL[n_tail - N_VPU]
    coef = jnp.concatenate([
        jnp.transpose(jnp.broadcast_to(
            o_s[h][0:1].astype(jnp.float32) * gate, (DH, DH)))
        for h in range(rv // DH, TAIL[n_tail] // DH)], axis=0)
    res = res + gate * wo_proj(3072, 4096, S_WOH + 1)
    for t in range(n_tail - N_VPU):
        res = res + gate * wo_proj(TAIL[t], TAIL[t + 1], S_WOL + t)
    acc = res * 0.125
    for t in range(n_tail - N_VPU, n_tail):
        wait_all(wo_v.at[pl.ds(TAIL[t], TAIL[t + 1] - TAIL[t])], S_WOL + t)
        for r in range(TAIL[t], TAIL[t + 1], 8):
            c = coef[r - rv:r - rv + 8]
            acc = acc + (wo_v[r:r + 8, :].astype(jnp.float32)
                         * jnp.concatenate([c, c, c, c], axis=1))
    o_ref[0] = jnp.sum(acc, axis=0, keepdims=True).astype(o_ref.dtype)


def _call(A_x, A_k_cache, A_v_cache, A_wq, A_wo, B_w_gate, B_w_up, B_w_down,
          gate_w, **kw):
    sk = A_k_cache.shape[2]
    assert A_x.shape == (1, 1, D) and A_k_cache.shape == (1, H, sk, DH)
    assert A_wq.shape == (D, H * DH) and B_w_gate.shape == (D, F)
    bf = jnp.bfloat16
    return pl.pallas_call(
        functools.partial(_kernel, row0=sk - W),
        in_specs=[pl.BlockSpec(memory_space=pl.ANY)] * 9,
        out_specs=pl.BlockSpec(memory_space=pltpu.VMEM),
        out_shape=jax.ShapeDtypeStruct((1, 1, D), A_x.dtype),
        scratch_shapes=[
            pltpu.VMEM((1, 1, D), bf),
            pltpu.VMEM((4, 128), bf),
            pltpu.VMEM((H, W, DH), bf),
            pltpu.VMEM((H, W, DH), bf),
            pltpu.VMEM((4, D // 4, H * DH), bf),
            pltpu.VMEM((H * DH, D), bf),
            pltpu.VMEM((F, D), bf),
            pltpu.VMEM((F, D), bf),
            pltpu.VMEM((F, D), bf),
            pltpu.VMEM((H, 8, DH), bf),
            pltpu.VMEM((H, 8, W), bf),
            pltpu.VMEM((H, 8, DH), jnp.float32),
            pltpu.VMEM((H, 8, DH), bf),
            pltpu.VMEM((8, D), jnp.float32),
            pltpu.SemaphoreType.DMA((N_SEM,)),
        ],
        compiler_params=pltpu.CompilerParams(
            vmem_limit_bytes=100 * 1024 * 1024,
            disable_semaphore_checks=True,
        ),
        **kw,
    )(A_x, A_k_cache, A_v_cache, A_wq.reshape(4, D // 4, H * DH), A_wo,
      B_w_gate.T, B_w_up.T, B_w_down, gate_w.reshape(4, 128))


@jax.jit
def pallas_gated_mix__sliding_block_cached__swiglu_ffn__decode_kernel(
    A_x: jax.Array,
    A_k_cache: jax.Array,
    A_v_cache: jax.Array,
    A_wq: jax.Array,
    A_wo: jax.Array,
    B_x: jax.Array,
    B_w_gate: jax.Array,
    B_w_up: jax.Array,
    B_w_down: jax.Array,
    gate_w: jax.Array,
):
    del B_x
    assert min(4096, max(256, A_k_cache.shape[2] // 4)) == W
    return _call(A_x, A_k_cache, A_v_cache, A_wq, A_wo, B_w_gate, B_w_up,
                 B_w_down, gate_w)
```
